```python
import jax
import jax.numpy as jnp

def _softmax(x, axis=-1):
    return jax.nn.softmax(x, axis=axis)
def _gelu(x):
    return jax.nn.gelu(x, approximate=True)
def _silu(x):
    return jax.nn.silu(x)
def _sigmoid(x):
    return jax.nn.sigmoid(x)
def _layernorm(x, axis=-1, eps=1e-5):
    m = jnp.mean(x, axis=axis, keepdims=True)
    v = jnp.var(x, axis=axis, keepdims=True)
    return (x - m) / jnp.sqrt(v + eps)
def _scatter_add(tgt, idx, src, axis=0):
    return tgt.at[idx].add(src)
def _segment_sum(src, seg, n):
    return jax.ops.segment_sum(src, seg, n)
class _Rng:
    def __init__(self, key):
        self._k = key
    def _next(self):
        self._k, sub = jax.random.split(self._k)
        return sub
    def normal(self, shape):
        return jax.random.normal(self._next(), shape, dtype=jnp.bfloat16)
    def randint(self, lo, hi, shape):
        return jax.random.randint(self._next(), shape, lo, hi, dtype=jnp.int32)
    def uniform(self, shape, lo=0.0, hi=1.0):
        return jax.random.uniform(self._next(), shape, jnp.bfloat16, lo, hi)
    def permutation(self, n):
        return jax.random.permutation(self._next(), n)


kernel_name = 'recurrent_scan__sliding_block_cached__glu_gated_glu__decode'

def setup_inputs():
    _rng = _Rng(jax.random.key(int.from_bytes(__import__("os").urandom(4), "little")))
    _w = (lambda a: (lambda t: t.astype(jnp.bfloat16) if jnp.issubdtype(t.dtype, jnp.floating) else t)(jnp.asarray(a)))
    def _A_setup():
        B, Sq, D = 1, 1, 576
        Hq, Hkv, Sk, Dh = 32, 16, 65536, 128
        assert Hq % Hkv == 0, (Hq, Hkv)
        return {
            "x": _w((lambda *s: _rng.normal(s) * 0.05)(B, Sq, D)),
            "k_cache": _w((lambda *s: _rng.normal(s) * 0.05)(B, Hkv, Sk, Dh)),
            "v_cache": _w((lambda *s: _rng.normal(s) * 0.05)(B, Hkv, Sk, Dh)),
            "wq": _w((lambda *s: _rng.normal(s) * 0.05)(D, Hq * Dh) * (D ** -0.5)),
            "wo": _w((lambda *s: _rng.normal(s) * 0.05)(Hq * Dh, D) * ((Hq * Dh) ** -0.5)),
        }
    _A_in = _A_setup()

    def _B_setup():
        B, S, D, F = 1, 1, 576, 4608
        return {
            "x": _w((lambda *s: _rng.normal(s) * 0.05)(B, S, D)),
            "w_gate": _w((lambda *s: _rng.normal(s) * 0.05)(D, F)),
            "w_up": _w((lambda *s: _rng.normal(s) * 0.05)(D, F)),
            "w_down": _w((lambda *s: _rng.normal(s) * 0.05)(F, D)),
        }
    _B_in = _B_setup()

    return {
        "A_x": _A_in["x"],
        "A_k_cache": _A_in["k_cache"],
        "A_v_cache": _A_in["v_cache"],
        "A_wq": _A_in["wq"],
        "A_wo": _A_in["wo"],
        "B_x": _B_in["x"],
        "B_w_gate": _B_in["w_gate"],
        "B_w_up": _B_in["w_up"],
        "B_w_down": _B_in["w_down"],
    }

def reference(A_x, A_k_cache, A_v_cache, A_wq, A_wo, B_x, B_w_gate, B_w_up, B_w_down):
    def _A_ref(x, k_cache, v_cache, wq, wo):
        B, Sq, D = x.shape
        Hq, Dh = 32, 128
        Hkv, Sk = k_cache.shape[1], k_cache.shape[2]
        W = min(4096, max(256, Sk // 4))
        rep = Hq // Hkv
        q = (lambda x, *d: x.transpose(*d))((x @ wq).reshape(B, Sq, Hq, Dh), 0, 2, 1, 3)
        k = jnp.repeat(k_cache[:, :, Sk - W:, :], rep, axis=1)
        v = jnp.repeat(v_cache[:, :, Sk - W:, :], rep, axis=1)
        scores = jnp.einsum("bhqd,bhkd->bhqk", q, k) * (Dh ** -0.5)
        p = _softmax(scores, axis=-1)
        o = jnp.einsum("bhqk,bhkd->bhqd", p, v)
        return (lambda x, *d: x.transpose(*d))(o, 0, 2, 1, 3).reshape(B, Sq, Hq * Dh) @ wo

    def _B_ref(x, w_gate, w_up, w_down):
        g = jnp.einsum("bsd,df->bsf", x, w_gate)
        u = jnp.einsum("bsd,df->bsf", x, w_up)
        h = _sigmoid(g) * u
        return jnp.einsum("bsf,fd->bsd", h, w_down)

    x = A_x
    xn = _layernorm(x, axis=-1)
    s = _A_ref(xn, A_k_cache, A_v_cache, A_wq, A_wo)
    g = _silu(_B_ref(xn, B_w_gate, B_w_up, B_w_down))
    return x + s * g
```

```python
import jax
import jax.numpy as jnp
from jax import lax
import jax.experimental.pallas as pl
import jax.experimental.pallas.tpu as pltpu

_HQ, _DH = 32, 128
_NT = (((1,), (1,)), ((), ()))
_WINDOW = 4
_F_CHUNKS = 4
_WO_CHUNKS = (1024, 1024, 1024, 512, 256, 128, 128)


def _kernel(x_hbm, k_hbm, v_hbm, wq_hbm, wo_hbm, wg_hbm, wu_hbm, wd_hbm, o_ref,
            kb, vb, wqb, wob, wgb, wub, wdb, xs, sems, xsem):
    hkv, win, dh = kb.shape
    d, f = wgb.shape
    fc = f // _F_CHUNKS
    s0 = k_hbm.shape[2] - win

    index, copies = {}, []

    def add(name, src, dst):
        index[name] = len(copies)
        copies.append(pltpu.make_async_copy(src, dst, sems.at[len(copies) % _WINDOW]))

    add("q", wq_hbm, wqb)
    for i in range(_F_CHUNKS):
        for name, src, dst in (("g", wg_hbm, wgb), ("u", wu_hbm, wub), ("d", wd_hbm, wdb)):
            add((name, i), src.at[:, pl.ds(i * fc, fc)], dst.at[:, pl.ds(i * fc, fc)])
    for h in range(hkv):
        add(("k", h), k_hbm.at[0, h, pl.ds(s0, win)], kb.at[h])
        add(("v", h), v_hbm.at[0, h, pl.ds(s0, win)], vb.at[h])
    off = 0
    for i, c in enumerate(_WO_CHUNKS):
        add(("o", i), wo_hbm.at[:, pl.ds(off, c)], wob.at[:, pl.ds(off, c)])
        off += c

    def wait(name):
        i = index[name]
        copies[i].wait()
        if i + _WINDOW < len(copies):
            copies[i + _WINDOW].start()

    x_copy = pltpu.make_async_copy(x_hbm, xs, xsem)
    copies[0].start()
    x_copy.start()
    for i in range(1, _WINDOW):
        copies[i].start()
    x_copy.wait()

    x = xs[0].astype(jnp.float32)
    xc = x - jnp.mean(x, axis=-1, keepdims=True)
    var = jnp.mean(xc * xc, axis=-1, keepdims=True)
    xn = jnp.broadcast_to(xc / jnp.sqrt(var + 1e-5), (8, d)).astype(jnp.bfloat16)

    wait("q")
    q = jnp.dot(xn, wqb[...], preferred_element_type=jnp.float32).astype(jnp.bfloat16)
    row = lax.broadcasted_iota(jnp.int32, (8, dh), 0)
    qs = [jnp.where(row == 0, q[:, 2 * h * dh:(2 * h + 1) * dh],
                    q[:, (2 * h + 1) * dh:(2 * h + 2) * dh]) for h in range(hkv)]

    y = jnp.zeros((8, d), jnp.float32)
    for i in range(_F_CHUNKS):
        cols = slice(i * fc, (i + 1) * fc)
        wait(("g", i))
        g = jnp.dot(xn, wgb[:, cols], preferred_element_type=jnp.float32)
        wait(("u", i))
        u = jnp.dot(xn, wub[:, cols], preferred_element_type=jnp.float32)
        hid = (jax.nn.sigmoid(g) * u).astype(jnp.bfloat16)
        wait(("d", i))
        y = y + lax.dot_general(hid, wdb[:, cols], _NT, preferred_element_type=jnp.float32)
    gate = y * jax.nn.sigmoid(y)

    heads = []
    for h in range(hkv):
        wait(("k", h))
        s = lax.dot_general(qs[h], kb[h], _NT, preferred_element_type=jnp.float32)
        s = s * (dh ** -0.5)
        p = jnp.exp(s - jnp.max(s, axis=-1, keepdims=True))
        l = jnp.sum(p, axis=-1, keepdims=True)
        wait(("v", h))
        o = jnp.dot(p.astype(jnp.bfloat16), vb[h], preferred_element_type=jnp.float32) / l
        heads.append(jnp.broadcast_to(o[0:1], (8, dh)).astype(jnp.bfloat16))
        heads.append(jnp.broadcast_to(o[1:2], (8, dh)).astype(jnp.bfloat16))

    s = jnp.zeros((8, d), jnp.float32)
    off = 0
    for i, c in enumerate(_WO_CHUNKS):
        lhs = jnp.concatenate(heads[off // dh:(off + c) // dh], axis=1)
        wait(("o", i))
        s = s + lax.dot_general(lhs, wob[:, off:off + c], _NT, preferred_element_type=jnp.float32)
        off += c
    o_ref[0] = (x + s[0:1] * gate[0:1]).astype(o_ref.dtype)


@jax.jit
def pallas_recurrent_scan__sliding_block_cached__glu_gated_glu__decode_kernel(
    A_x: jax.Array,
    A_k_cache: jax.Array,
    A_v_cache: jax.Array,
    A_wq: jax.Array,
    A_wo: jax.Array,
    B_x: jax.Array,
    B_w_gate: jax.Array,
    B_w_up: jax.Array,
    B_w_down: jax.Array,
):
    del B_x
    _, hkv, sk, dh = A_k_cache.shape
    win = min(4096, max(256, sk // 4))
    d, f = B_w_gate.shape
    assert A_x.shape == (1, 1, d) and dh == _DH and 2 * hkv == _HQ
    hbm = pl.BlockSpec(memory_space=pltpu.HBM)
    return pl.pallas_call(
        _kernel,
        out_shape=jax.ShapeDtypeStruct(A_x.shape, A_x.dtype),
        in_specs=[hbm] * 8,
        out_specs=pl.BlockSpec(memory_space=pltpu.VMEM),
        scratch_shapes=[
            pltpu.VMEM((hkv, win, dh), A_k_cache.dtype),
            pltpu.VMEM((hkv, win, dh), A_v_cache.dtype),
            pltpu.VMEM((d, _HQ * dh), A_wq.dtype),
            pltpu.VMEM((d, _HQ * dh), A_wo.dtype),
            pltpu.VMEM((d, f), B_w_gate.dtype),
            pltpu.VMEM((d, f), B_w_up.dtype),
            pltpu.VMEM((d, f), B_w_down.dtype),
            pltpu.VMEM(A_x.shape, A_x.dtype),
            pltpu.SemaphoreType.DMA((_WINDOW,)),
            pltpu.SemaphoreType.DMA(()),
        ],
        compiler_params=pltpu.CompilerParams(vmem_limit_bytes=100 * 1024 * 1024),
    )(A_x, A_k_cache, A_v_cache, A_wq, A_wo.T, B_w_gate, B_w_up, B_w_down.T)
```

```python
import jax
import jax.numpy as jnp
from jax import lax
import jax.experimental.pallas as pl
import jax.experimental.pallas.tpu as pltpu

_HQ, _DH = 32, 128
_NT = (((1,), (1,)), ((), ()))
_WINDOW = 3
_F_CHUNKS = 2
_WO_PIECES = (
    (0, 256, (4096,)),
    (256, 384, (4096,)),
    (384, 512, (4096,)),
    (512, 576, (2048, 1024, 1024)),
)


def _stream_and_compute(x_hbm, k_hbm, v_hbm, wq_hbm, wo_hbm, wg_hbm, wu_hbm, wd_hbm,
                        kb, vb, wqb, wob, wgb, wub, wdb, xs, outs, sems, xsem):
    hkv, win, dh = kb.shape
    d, f = wgb.shape
    fc = f // _F_CHUNKS
    s0 = k_hbm.shape[2] - win

    index, copies = {}, []

    def add(name, src, dst):
        index[name] = len(copies)
        copies.append(pltpu.make_async_copy(src, dst, sems.at[len(copies) % _WINDOW]))

    add("q", wq_hbm, wqb)
    for i in range(_F_CHUNKS):
        for name, src, dst in (("g", wg_hbm, wgb), ("u", wu_hbm, wub), ("d", wd_hbm, wdb)):
            add((name, i), src.at[:, pl.ds(i * fc, fc)], dst.at[:, pl.ds(i * fc, fc)])
    for h in range(hkv):
        add(("k", h), k_hbm.at[0, h, pl.ds(s0, win)], kb.at[h])
        add(("v", h), v_hbm.at[0, h, pl.ds(s0, win)], vb.at[h])
    for i, (r0, r1, widths) in enumerate(_WO_PIECES):
        off = 0
        for j, c in enumerate(widths):
            piece = (pl.ds(r0, r1 - r0), pl.ds(off, c))
            add(("o", i, j), wo_hbm.at[piece], wob.at[piece])
            off += c

    def wait(name):
        i = index[name]
        copies[i].wait()
        if i + _WINDOW < len(copies):
            copies[i + _WINDOW].start()

    x_copy = pltpu.make_async_copy(x_hbm, xs, xsem)
    copies[0].start()
    x_copy.start()
    for i in range(1, _WINDOW):
        copies[i].start()
    x_copy.wait()

    x = xs[0].astype(jnp.float32)
    xc = x - jnp.mean(x, axis=-1, keepdims=True)
    var = jnp.mean(xc * xc, axis=-1, keepdims=True)
    xn = jnp.broadcast_to(xc / jnp.sqrt(var + 1e-5), (8, d)).astype(jnp.bfloat16)

    wait("q")
    q = jnp.dot(xn, wqb[...], preferred_element_type=jnp.float32).astype(jnp.bfloat16)
    row = lax.broadcasted_iota(jnp.int32, (8, dh), 0)
    qs = [jnp.where(row == 0, q[:, 2 * h * dh:(2 * h + 1) * dh],
                    q[:, (2 * h + 1) * dh:(2 * h + 2) * dh]) for h in range(hkv)]

    y = jnp.zeros((8, d), jnp.float32)
    for i in range(_F_CHUNKS):
        cols = slice(i * fc, (i + 1) * fc)
        wait(("g", i))
        g = jnp.dot(xn, wgb[:, cols], preferred_element_type=jnp.float32)
        wait(("u", i))
        u = jnp.dot(xn, wub[:, cols], preferred_element_type=jnp.float32)
        hid = (jax.nn.sigmoid(g) * u).astype(jnp.bfloat16)
        wait(("d", i))
        y = y + lax.dot_general(hid, wdb[:, cols], _NT, preferred_element_type=jnp.float32)
    gate = y * jax.nn.sigmoid(y)

    heads = []
    for h in range(hkv):
        wait(("k", h))
        s = lax.dot_general(qs[h], kb[h], _NT, preferred_element_type=jnp.float32)
        s = s * (dh ** -0.5)
        p = jnp.exp(s - jnp.max(s, axis=-1, keepdims=True))
        l = jnp.sum(p, axis=-1, keepdims=True)
        wait(("v", h))
        o = jnp.dot(p.astype(jnp.bfloat16), vb[h], preferred_element_type=jnp.float32) / l
        heads.append(jnp.broadcast_to(o[0:1], (8, dh)).astype(jnp.bfloat16))
        heads.append(jnp.broadcast_to(o[1:2], (8, dh)).astype(jnp.bfloat16))

    for i, (r0, r1, widths) in enumerate(_WO_PIECES):
        s = jnp.zeros((8, r1 - r0), jnp.float32)
        off = 0
        for j, c in enumerate(widths):
            lhs = jnp.concatenate(heads[off // dh:(off + c) // dh], axis=1)
            wait(("o", i, j))
            s = s + lax.dot_general(lhs, wob[r0:r1, off:off + c], _NT,
                                    preferred_element_type=jnp.float32)
            off += c
        outs[0, :, r0:r1] = (x[:, r0:r1] + s[0:1] * gate[0:1, r0:r1]).astype(outs.dtype)


def _kernel(*refs):
    ins, o_hbm, bufs, osem = refs[:8], refs[8], refs[9:-1], refs[-1]
    out_copy = pltpu.make_async_copy(bufs[-1], o_hbm, osem)

    def scoped(sems, xsem):
        _stream_and_compute(*ins, *bufs, sems, xsem)
        out_copy.start()

    pl.run_scoped(scoped, pltpu.SemaphoreType.DMA((_WINDOW,)), pltpu.SemaphoreType.DMA(()))
    out_copy.wait()


@jax.jit
def pallas_recurrent_scan__sliding_block_cached__glu_gated_glu__decode_kernel(
    A_x: jax.Array,
    A_k_cache: jax.Array,
    A_v_cache: jax.Array,
    A_wq: jax.Array,
    A_wo: jax.Array,
    B_x: jax.Array,
    B_w_gate: jax.Array,
    B_w_up: jax.Array,
    B_w_down: jax.Array,
):
    del B_x
    _, hkv, sk, dh = A_k_cache.shape
    win = min(4096, max(256, sk // 4))
    d, f = B_w_gate.shape
    assert A_x.shape == (1, 1, d) and d == _WO_PIECES[-1][1]
    assert dh == _DH and 2 * hkv == _HQ
    hbm = pl.BlockSpec(memory_space=pltpu.HBM)
    return pl.pallas_call(
        _kernel,
        out_shape=jax.ShapeDtypeStruct(A_x.shape, A_x.dtype),
        in_specs=[hbm] * 8,
        out_specs=hbm,
        scratch_shapes=[
            pltpu.VMEM((hkv, win, dh), A_k_cache.dtype),
            pltpu.VMEM((hkv, win, dh), A_v_cache.dtype),
            pltpu.VMEM((d, _HQ * dh), A_wq.dtype),
            pltpu.VMEM((d, _HQ * dh), A_wo.dtype),
            pltpu.VMEM((d, f), B_w_gate.dtype),
            pltpu.VMEM((d, f), B_w_up.dtype),
            pltpu.VMEM((d, f), B_w_down.dtype),
            pltpu.VMEM(A_x.shape, A_x.dtype),
            pltpu.VMEM(A_x.shape, A_x.dtype),
            pltpu.SemaphoreType.DMA(()),
        ],
        compiler_params=pltpu.CompilerParams(vmem_limit_bytes=100 * 1024 * 1024),
    )(A_x, A_k_cache, A_v_cache, A_wq, A_wo.T, B_w_gate, B_w_up, B_w_down.T)
```
